```python
import os as _os
_os.environ.setdefault("JAX_PLATFORMS", "cpu")
import jax
import jax.numpy as jnp

def _softmax(x, axis=-1):
    return jax.nn.softmax(x, axis=axis)
def _gelu(x):
    return jax.nn.gelu(x, approximate=True)
def _silu(x):
    return jax.nn.silu(x)
def _sigmoid(x):
    return jax.nn.sigmoid(x)
def _layernorm(x, axis=-1, eps=1e-5):
    m = jnp.mean(x, axis=axis, keepdims=True)
    v = jnp.var(x, axis=axis, keepdims=True)
    return (x - m) / jnp.sqrt(v + eps)
def _scatter_add(tgt, idx, src, axis=0):
    return tgt.at[idx].add(src)
def _segment_sum(src, seg, n):
    return jax.ops.segment_sum(src, seg, n)
class _Rng:
    def __init__(self, key):
        self._k = key
    def _next(self):
        self._k, sub = jax.random.split(self._k)
        return sub
    def normal(self, shape):
        return jax.random.normal(self._next(), shape, dtype=jnp.bfloat16)
    def randint(self, lo, hi, shape):
        return jax.random.randint(self._next(), shape, lo, hi, dtype=jnp.int32)
    def uniform(self, shape, lo=0.0, hi=1.0):
        return jax.random.uniform(self._next(), shape, jnp.bfloat16, lo, hi)
    def permutation(self, n):
        return jax.random.permutation(self._next(), n)


kernel_name = 'gated_mix__spectral_gfnet__dense_activation_silu__prompt'

def setup_inputs():
    _rng = _Rng(jax.random.key(int.from_bytes(__import__("os").urandom(4), "little")))
    _w = (lambda a: (lambda t: t.astype(jnp.bfloat16) if jnp.issubdtype(t.dtype, jnp.floating) else t)(jnp.asarray(a)))
    def _A_setup():
        B, S, D = 1, 2048, 512
        Df = D // 2 + 1
        return {
            "x": _w((lambda *s: _rng.normal(s) * 0.05)(B, S, D)),
            "w_r": _w((lambda *s: _rng.normal(s) * 0.05)(S, Df) * 0.02),
            "w_i": _w((lambda *s: _rng.normal(s) * 0.05)(S, Df) * 0.02),
        }
    _A_in = _A_setup()

    def _B_setup():
        B, S, D, F = 1, 2048, 512, 1376
        return {
            "x": _w((lambda *s: _rng.normal(s) * 0.05)(B, S, D)),
            "w1": _w((lambda *s: _rng.normal(s) * 0.05)(D, F) * (D ** -0.5)),
            "w2": _w((lambda *s: _rng.normal(s) * 0.05)(F, D) * (F ** -0.5)),
        }
    _B_in = _B_setup()

    return {
        "A_x": _A_in["x"],
        "A_w_r": _A_in["w_r"],
        "A_w_i": _A_in["w_i"],
        "B_x": _B_in["x"],
        "B_w1": _B_in["w1"],
        "B_w2": _B_in["w2"],
        "gate_w": _w((lambda *s: _rng.normal(s) * 0.05)(512) * 16.0),
    }

def reference(A_x, A_w_r, A_w_i, B_x, B_w1, B_w2, gate_w):
    def _A_ref(x, w_r, w_i):
        B, S, D = x.shape
        X = (lambda x, axes=(-2,-1): jnp.fft.rfft2(x.astype(jnp.float32), axes=axes))(x, axes=(-2, -1))
        W = w_r + 1j * w_i
        X = X * W
        y = (lambda x, s, axes=(-2,-1): jnp.fft.irfft2(x, s=s, axes=axes).astype(jnp.bfloat16))(X, (S, D), axes=(-2, -1))
        return y

    def _B_ref(x, w1, w2):
        h = jnp.einsum("bsd,df->bsf", x, w1)
        h = _silu(h)
        out = jnp.einsum("bsf,fd->bsd", h, w2)
        return out

    x = A_x
    g = _sigmoid((x * gate_w).sum(-1, keepdims=True))
    a = _A_ref(x, A_w_r, A_w_i)
    b = _B_ref(x, B_w1, B_w2)
    return g * a + (1 - g) * b
```

```python
import jax
import jax.numpy as jnp
import numpy as np
import jax.experimental.pallas as pl
import jax.experimental.pallas.tpu as pltpu

S, D, F = 2048, 512, 1376
KR = 264
f32, bf16 = jnp.float32, jnp.bfloat16


def _consts():
    n = np.arange(128)
    m = np.arange(64)
    th = lambda k, t: 2 * np.pi * np.outer(k, t) / D
    a0 = th(4 * m, n)
    f0 = np.concatenate([np.cos(a0), -np.sin(a0)])
    f0[64] = (-1.0) ** n
    g0 = 2 * f0
    g0[0] /= 2
    g0[64] /= 2
    a2 = th(4 * m + 2, n)
    f2 = np.concatenate([np.cos(a2), -np.sin(a2)])
    a1, a3 = th(4 * m + 1, n), th(4 * m + 3, n)
    c1, s1, c3, s3 = np.cos(a1), np.sin(a1), np.cos(a3), np.sin(a3)
    cat = np.concatenate
    fo = cat([c1, c3, -(s1 + c1), s3 - c3, c1 - s1, -(s3 + c3)])
    sc = 1.0 / (S * D)
    fw = cat([f0, f2, fo])
    gm = cat([g0, 2 * f2, 2 * cat([c1, c3, c1 - s1, -(s3 + c3), -s1 - c1, s3 - c3])]) * sc
    ms = []
    for n1 in range(16):
        a = 2 * np.pi * (np.outer(n, n) / 128 + n1 * n[None, :] / S)
        c, s = np.cos(a), np.sin(a)
        ms.append(np.stack([c, s - c, c + s]))
    cast = lambda v: np.asarray(v, np.float32).astype(bf16)
    return cast(fw), cast(gm), cast(np.stack(ms))


def _fft16(v, sign):
    n = len(v)
    if n == 1:
        return v
    e, o = _fft16(v[0::2], sign), _fft16(v[1::2], sign)
    out = [None] * n
    for k in range(n // 2):
        (er, ei), (r, i) = e[k], o[k]
        c, s = float(np.cos(2 * np.pi * k / n)), float(sign * np.sin(2 * np.pi * k / n))
        if k == 0:
            tr, ti = r, i
        elif 4 * k == n:
            out[k] = (er - sign * i, ei + sign * r) if sign > 0 else (er + i, ei - r)
            out[k + n // 2] = (er + i, ei - r) if sign > 0 else (er - i, ei + r)
            continue
        elif 8 * k == n:
            tr, ti = ((r - i) * c, (r + i) * c) if sign > 0 else ((r + i) * c, (i - r) * c)
        elif 8 * k == 3 * n:
            tr, ti = ((r + i) * c, (i - r) * c) if sign > 0 else ((r - i) * c, (r + i) * c)
        else:
            tr, ti = r * c - i * s, r * s + i * c
        out[k] = (er + tr, ei + ti)
        out[k + n // 2] = (er - tr, ei - ti)
    return out


def _nt(a, b):
    return jax.lax.dot_general(a, b, (((1,), (1,)), ((), ())), preferred_element_type=f32)


def _lo(w):
    return pltpu.bitcast(w << 16, f32)


def _hi(w):
    return pltpu.bitcast(w & jnp.uint32(0xFFFF0000), f32)


def _nn(a, b):
    return jnp.dot(a, b, preferred_element_type=f32)


def _kernel(x_h, wr_h, wi_h, w1_h, w2_h, gw_h, fw_h, gm_h, m_h, o_h,
            wr, wi, xb, w1, w2, gw, fw, gm, mm, u, z, yb, gs, ob, xs, ws, nr, ni, sem, osem):
    col = lambda h, v: [(h.at[0:256, t * 128:(t + 1) * 128], v[t]) for t in range(16)]
    pairs = ([(x_h.at[0:256], xb.at[0:256]), (w1_h, w1), (w2_h, w2), (gw_h, gw),
              (x_h.at[256:S], xb.at[256:S]), (fw_h, fw)]
             + [(m_h.at[4 * i:4 * i + 4], mm.at[4 * i:4 * i + 4]) for i in range(4)]
             + col(wr_h, wr) + col(wi_h, wi)
             + [(wr_h.at[256:257], nr), (wi_h.at[256:257], ni), (gm_h, gm)])
    cps = [pltpu.make_async_copy(a, b, sem.at[i]) for i, (a, b) in enumerate(pairs)]
    row = jax.lax.broadcasted_iota(jnp.int32, (8, 128), 0)

    def ffn(r, n, other=()):
        other = list(other)
        x = xb[pl.ds(r, n), :]
        sl = []
        for c in range(0, F, 384):
            e = min(c + 384, F)
            hh = 0.5 * _nt(x, w1[c:e])
            sl.append((hh * jnp.tanh(hh) + hh).astype(bf16))
            if other:
                other.pop(0)()
        acc = 0.0
        for i, c in enumerate(range(0, F, 384)):
            acc = acc + _nn(sl[i], w2[c:min(c + 384, F)])
            if other:
                other.pop(0)()
        g = jax.nn.sigmoid(jnp.sum(x.astype(f32) * gw[...].astype(f32), -1, keepdims=True))
        gs[pl.ds(r, n), :] = jnp.broadcast_to(g, (n, 128))
        yb[pl.ds(r, n), :] = (1 - g) * acc

    def fwd(p):
        w = [xs[t, pl.ds(p, 128, stride=8), :] for t in range(4)]
        for h, part in enumerate((_lo, _hi)):
            x0, x1, x2, x3 = [part(t) for t in w]
            s0, s1, p_, q_ = x0 + x2, x1 + x3, x0 - x2, x1 - x3
            r0 = _nt(fw[0:128], (s0 + s1).astype(bf16))
            r2 = _nt(fw[128:256], (s0 - s1).astype(bf16))
            t1 = _nt(fw[256:384], (p_ + q_).astype(bf16))
            ro = t1 + _nt(fw[384:512], q_.astype(bf16))
            t3 = _nt(fw[512:640], p_.astype(bf16))
            nyq = jnp.where(row == 0, r0[64:72], 0.0)
            i00 = jnp.where(row == 0, 0.0, r0[64:72])
            zero = jnp.zeros((8, 128), f32)
            re = jnp.concatenate([r0[0:64], ro[0:64], r2[0:64], ro[64:128], nyq, zero], 0)
            im = jnp.concatenate([i00, r0[72:128], t3[0:64] - t1[0:64], r2[64:128],
                                  t3[64:128] + t1[64:128], zero, zero], 0)
            j = 2 * p + h
            k1 = _nn((re + im).astype(bf16), mm[j, 0])
            u[j, :, 0:128] = (k1 + _nn(im.astype(bf16), mm[j, 1]))[0:KR]
            u[j, :, 128:256] = (k1 - _nn(re.astype(bf16), mm[j, 2]))[0:KR]

    def spec(r, getw):
        v = [(u[j, pl.ds(r, 8), 0:128], u[j, pl.ds(r, 8), 128:256]) for j in range(16)]
        v = _fft16(v, -1)
        y = []
        for k1, (a, b) in enumerate(v):
            c, d = getw(wr, k1), getw(wi, k1)
            y.append((a * c - b * d, a * d + b * c))
        for j, (a, b) in enumerate(_fft16(y, 1)):
            u[j, pl.ds(r, 8), 0:128] = a
            u[j, pl.ds(r, 8), 128:256] = b

    def inv(j):
        yr, yi = u[j, :, 0:128], u[j, :, 128:256]
        k1 = _nt((yr + yi).astype(bf16), mm[j, 0])
        re = k1 - _nt(yi.astype(bf16), mm[j, 2])
        im = k1 + _nt(yr.astype(bf16), mm[j, 1])
        i00 = jnp.where(row == 0, re[256:264], im[0:8])
        tiles = [jnp.concatenate([re[0:64], i00, im[8:64]], 0),
                 jnp.concatenate([re[128:192], im[128:192]], 0),
                 jnp.concatenate([re[64:128], re[192:256]], 0),
                 jnp.concatenate([im[64:128], im[192:256]], 0)]
        for t in range(4):
            z[t, pl.ds(j, 128, stride=16), :] = tiles[t].T

    sign = jnp.where(jax.lax.broadcasted_iota(jnp.int32, (1, 128), 1) < 64, -1.0, 1.0)

    def fin(b):
        r = pl.ds(b * 256, 256)
        re, im = z[2, r, :], z[3, r, :]
        e0 = _nn(z[0, r, :].astype(bf16), gm[0:128])
        e2 = _nn(z[1, r, :].astype(bf16), gm[128:256])
        t1 = _nn((re + sign * im).astype(bf16), gm[256:384])
        o0 = t1 + _nn(im.astype(bf16), gm[384:512])
        o1 = t1 + _nn(re.astype(bf16), gm[512:640])
        s0, s1, g = e0 + e2, e0 - e2, gs[r, :]
        a = jnp.concatenate([g * (s0 + o0), g * (s1 + o1), g * (s0 - o0), g * (s1 - o1)], 1)
        ob[r, :] = (a + yb[r, :]).astype(bf16)
        c = pltpu.make_async_copy(ob.at[r], o_h.at[r], osem.at[b])
        c.start()
        return c

    cps[0].start()
    cps[1].start()
    cps[1].wait()
    for c in cps[2:4]:
        c.start()
    cps[0].wait()
    cps[3].wait()
    cps[2].wait()
    for c in cps[4:7]:
        c.start()
    ffn(0, 256)
    cps[4].wait()
    for c in cps[7:]:
        c.start()
    cps[5].wait()
    for t in range(4):
        xs[t] = pltpu.bitcast(xb[:, t * 128:(t + 1) * 128], jnp.uint32)

    def front(t, _):
        pltpu.make_async_copy(m_h.at[pl.ds(4 * t, 4)], mm.at[pl.ds(4 * t, 4)], sem.at[6 + t]).wait()
        ffn(pl.multiple_of(256 + t * 128, 128), 128,
            [lambda: None, lambda: fwd(2 * t), lambda: None, lambda: None, lambda: None,
             lambda: fwd(2 * t + 1)])
        return _

    jax.lax.fori_loop(0, 4, front, 0)
    for c in cps[10:44]:
        c.wait()
    for t, a in enumerate(list(wr) + list(wi)):
        ws[t] = pltpu.bitcast(a[...], jnp.uint32)

    def mid(t, _):
        def one(i, g):
                part = _hi if g % 2 else _lo
                spec(pl.multiple_of(g * 64 + t * 16 + i * 8, 8),
                     lambda ref, k1: part(ws[(0 if ref is wr else 16) + k1,
                                             pl.ds(32 * t + 16 * i + g // 2, 8, stride=2), :]))

        ffn(pl.multiple_of(768 + t * 128, 128), 128,
            [lambda i=i, g=g: one(i, g) for i in range(2) for g in range(4)])
        return _

    jax.lax.fori_loop(0, 4, mid, 0)
    spec(256, lambda ref, k1: (nr if ref is wr else ni)[:, k1 * 128:(k1 + 1) * 128].astype(f32))

    def back(t, _):
        ffn(pl.multiple_of(1280 + t * 128, 128), 128,
            [(lambda i=i: inv(4 * t + i // 2)) if i % 2 == 0 else (lambda: None)
             for i in range(8)])
        return _

    jax.lax.fori_loop(0, 4, back, 0)
    cps[44].wait()
    outs = []
    for b in range(8):
        if b in (0, 3):
            ffn(1792 + b // 3 * 128, 128)
        outs.append(fin(b))
    for c in outs:
        c.wait()


@jax.jit
def pallas_gated_mix__spectral_gfnet__dense_activation_silu__prompt_kernel(
        A_x, A_w_r, A_w_i, B_x, B_w1, B_w2, gate_w):
    ins = [A_x.reshape(S, D), A_w_r.T, A_w_i.T, B_w1.T, B_w2,
           gate_w.reshape(1, D)] + [jnp.asarray(c) for c in _consts()]
    vm = pltpu.VMEM
    scratch = [[vm((256, 128), bf16)] * 16] * 2 + [vm((S, D), bf16)] + [
        vm(a.shape, a.dtype) for a in ins[3:]] + [
        vm((16, KR, 256), f32), vm((4, S, 128), f32), vm((S, D), f32), vm((S, 128), f32),
        vm((S, D), bf16), vm((4, 1024, 128), jnp.uint32), vm((32, 128, 128), jnp.uint32),
        vm((1, S), bf16), vm((1, S), bf16),
        pltpu.SemaphoreType.DMA((45,)), pltpu.SemaphoreType.DMA((8,))]
    out = pl.pallas_call(
        _kernel,
        in_specs=[pl.BlockSpec(memory_space=pltpu.HBM)] * len(ins),
        out_specs=pl.BlockSpec(memory_space=pltpu.HBM),
        out_shape=jax.ShapeDtypeStruct((S, D), bf16),
        scratch_shapes=scratch,
        compiler_params=pltpu.CompilerParams(vmem_limit_bytes=100 << 20),
    )(*ins)
    return out.reshape(1, S, D)
```
